```python
import os as _os
_os.environ.setdefault("JAX_PLATFORMS", "cpu")
import jax
import jax.numpy as jnp

def _softmax(x, axis=-1):
    return jax.nn.softmax(x, axis=axis)
def _gelu(x):
    return jax.nn.gelu(x, approximate=True)
def _silu(x):
    return jax.nn.silu(x)
def _sigmoid(x):
    return jax.nn.sigmoid(x)
def _layernorm(x, axis=-1, eps=1e-5):
    m = jnp.mean(x, axis=axis, keepdims=True)
    v = jnp.var(x, axis=axis, keepdims=True)
    return (x - m) / jnp.sqrt(v + eps)
def _scatter_add(tgt, idx, src, axis=0):
    return tgt.at[idx].add(src)
def _segment_sum(src, seg, n):
    return jax.ops.segment_sum(src, seg, n)
class _Rng:
    def __init__(self, key):
        self._k = key
    def _next(self):
        self._k, sub = jax.random.split(self._k)
        return sub
    def normal(self, shape):
        return jax.random.normal(self._next(), shape, dtype=jnp.bfloat16)
    def randint(self, lo, hi, shape):
        return jax.random.randint(self._next(), shape, lo, hi, dtype=jnp.int32)
    def uniform(self, shape, lo=0.0, hi=1.0):
        return jax.random.uniform(self._next(), shape, jnp.bfloat16, lo, hi)
    def permutation(self, n):
        return jax.random.permutation(self._next(), n)


kernel_name = 'concat_heads__mha_block_cached__gqa_block_cached__decode'

def setup_inputs():
    _rng = _Rng(jax.random.key(int.from_bytes(__import__("os").urandom(4), "little")))
    _w = (lambda a: (lambda t: t.astype(jnp.bfloat16) if jnp.issubdtype(t.dtype, jnp.floating) else t)(jnp.asarray(a)))
    def _A_setup():
        B, Sq, D = 1, 1, 512
        H, Sk, Dh = 32, 4096, 128
        return {
            "x": _w((lambda *s: _rng.normal(s) * 0.8)(B, Sq, D)),
            "k_cache": _w((lambda *s: _rng.normal(s) * 0.8)(B, H, Sk, Dh)),
            "v_cache": _w((lambda *s: _rng.normal(s) * 0.05)(B, H, Sk, Dh)),
            "wq": _w((lambda *s: _rng.normal(s) * 0.8)(D, H * Dh) * (D ** -0.5)),
            "wo": _w((lambda *s: _rng.normal(s) * 0.05)(H * Dh, D) * ((H * Dh) ** -0.5)),
        }
    _A_in = _A_setup()

    def _B_setup():
        B, Sq, D = 1, 1, 512
        Hq, Hkv, Sk, Dh = 32, 32, 4096, 128
        assert Hq % Hkv == 0, (Hq, Hkv)
        return {
            "x": _w((lambda *s: _rng.normal(s) * 0.8)(B, Sq, D)),
            "k_cache": _w((lambda *s: _rng.normal(s) * 0.8)(B, Hkv, Sk, Dh)),
            "v_cache": _w((lambda *s: _rng.normal(s) * 0.05)(B, Hkv, Sk, Dh)),
            "wq": _w((lambda *s: _rng.normal(s) * 0.8)(D, Hq * Dh) * (D ** -0.5)),
            "wo": _w((lambda *s: _rng.normal(s) * 0.05)(Hq * Dh, D) * ((Hq * Dh) ** -0.5)),
        }
    _B_in = _B_setup()

    return {
        "A_x": _A_in["x"],
        "A_k_cache": _A_in["k_cache"],
        "A_v_cache": _A_in["v_cache"],
        "A_wq": _A_in["wq"],
        "A_wo": _A_in["wo"],
        "B_x": _B_in["x"],
        "B_k_cache": _B_in["k_cache"],
        "B_v_cache": _B_in["v_cache"],
        "B_wq": _B_in["wq"],
        "B_wo": _B_in["wo"],
    }

def reference(A_x, A_k_cache, A_v_cache, A_wq, A_wo, B_x, B_k_cache, B_v_cache, B_wq, B_wo):
    def _A_ref(x, k_cache, v_cache, wq, wo):
        B, Sq, D = x.shape
        H, Dh = 32, 128
        q = (lambda x, *d: x.transpose(*d))((x @ wq).reshape(B, Sq, H, Dh), 0, 2, 1, 3)
        scores = jnp.einsum("bhqd,bhkd->bhqk", q, k_cache) * (Dh ** -0.5)
        p = _softmax(scores, axis=-1)
        o = jnp.einsum("bhqk,bhkd->bhqd", p, v_cache)
        return (lambda x, *d: x.transpose(*d))(o, 0, 2, 1, 3).reshape(B, Sq, H * Dh) @ wo

    def _B_ref(x, k_cache, v_cache, wq, wo):
        B, Sq, D = x.shape
        Hq, Dh = 32, 128
        Hkv = k_cache.shape[1]
        rep = Hq // Hkv
        q = (lambda x, *d: x.transpose(*d))((x @ wq).reshape(B, Sq, Hq, Dh), 0, 2, 1, 3)
        k = jnp.repeat(k_cache, rep, axis=1)
        v = jnp.repeat(v_cache, rep, axis=1)
        scores = jnp.einsum("bhqd,bhkd->bhqk", q, k) * (Dh ** -0.5)
        p = _softmax(scores, axis=-1)
        o = jnp.einsum("bhqk,bhkd->bhqd", p, v)
        return (lambda x, *d: x.transpose(*d))(o, 0, 2, 1, 3).reshape(B, Sq, Hq * Dh) @ wo

    a = _A_ref(A_x, A_k_cache, A_v_cache, A_wq, A_wo)
    b = _B_ref(B_x, B_k_cache, B_v_cache, B_wq, B_wo)
    return jnp.concatenate([a, b], axis=-1)
```

```python
import functools
import jax
import jax.numpy as jnp
from jax import lax
import jax.experimental.pallas as pl
import jax.experimental.pallas.tpu as pltpu

T = 128
HG = 8
NT = (((1,), (1,)), ((), ()))


def make(depth=6, nslot=8, rows=16, compute=True):
    ng = T // rows

    def kernel(ax, ak, av, awq, awo, bx, bk, bv, bwq, bwo, out_ref,
               kvbuf, wqbuf, wobuf, xbuf, q_scr, s_scr, m_scr, o_scr, sem, xsem):
        H, S, _ = ak.shape
        D = awq.shape[0]
        G = H // HG
        NI = S // T
        ND = D // T
        n_q, n_kv, n_o = G * ND, G * NI, H // 2
        row = lax.broadcasted_iota(jnp.int32, (HG, T), 0)
        scale = T ** -0.5

        def slot_of(t):
            return lax.rem(t, nslot)

        def issue_wq(j, slot):
            g, r = j // ND, lax.rem(j, ND)
            for d in range(8):
                for b, w in enumerate((awq, bwq)):
                    r0 = pl.multiple_of(r * T + d * 16, 16)
                    c0 = pl.multiple_of(g * (HG * T), HG * T)
                    pltpu.make_async_copy(w.at[pl.ds(r0, 16), pl.ds(c0, HG * T)],
                                          wqbuf.at[slot, b, pl.ds(d * 16, 16)], sem.at[slot, b]).start(priority=b)

        def issue_kv(srcs, j, slot):
            g, i = j // NI, lax.rem(j, NI)
            for d in range(T // rows):
                for hh in range(HG // ng):
                    for b, a in enumerate(srcs):
                        r0 = pl.multiple_of(i * T + d * rows, rows)
                        pltpu.make_async_copy(a.at[pl.ds(g * HG + hh * ng, ng), pl.ds(r0, rows)],
                                              kvbuf.at[slot, b, pl.ds(hh * ng, ng), pl.ds(d * rows, rows)],
                                              sem.at[slot, b]).start(priority=b)

        def issue_wo(j, slot):
            for d in range(8):
                for b, w in enumerate((awo, bwo)):
                    r0 = pl.multiple_of(j * (2 * T) + d * 32, 32)
                    pltpu.make_async_copy(w.at[pl.ds(r0, 32)], wobuf.at[slot, b, pl.ds(d * 32, 32)],
                                          sem.at[slot, b]).start(priority=b)

        def wait(buf, slot):
            for b in range(2):
                pltpu.make_async_copy(buf.at[slot, b], buf.at[slot, b], sem.at[slot, b]).wait()

        def advance(j, n, base, issue_same, issue_next):
            slot = slot_of(base + j + depth)

            @pl.when(j + depth < n)
            def _():
                issue_same(j + depth, slot)

            if issue_next is not None:
                @pl.when(j + depth >= n)
                def _():
                    issue_next(j + depth - n, slot)

        issue_k = functools.partial(issue_kv, (ak, bk))
        issue_v = functools.partial(issue_kv, (av, bv))

        def pro(j, c):
            issue_wq(j, j)
            return c
        issue_wq(0, 0)
        xcp = [pltpu.make_async_copy(x, xbuf.at[b], xsem.at[b]) for b, x in enumerate((ax, bx))]
        for c in xcp:
            c.start()
        lax.fori_loop(1, depth, pro, 0)
        for c in xcp:
            c.wait()

        zero = jnp.zeros((HG, T), jnp.float32)

        def q_body(j, acc):
            slot = slot_of(j)
            wait(wqbuf, slot)
            advance(j, n_q, 0, issue_wq, issue_k)
            g, r = j // ND, lax.rem(j, ND)
            new = []
            for b in range(2):
                a = jnp.where(r == 0, 0.0, acc[b])
                if compute:
                    xr = xbuf[b, :, pl.ds(pl.multiple_of(r * T, T), T)]
                    x8 = jnp.broadcast_to(xr.astype(jnp.float32), (HG, T)).astype(jnp.bfloat16)
                    res = jnp.dot(x8, wqbuf[slot, b], preferred_element_type=jnp.float32)
                    sel = res[:, 0:T]
                    for h in range(1, HG):
                        sel = jnp.where(row == h, res[:, h * T:(h + 1) * T], sel)
                    a = a + sel
                q_scr[b, g] = a
                new.append(a)
            return tuple(new)
        lax.fori_loop(0, n_q, q_body, (zero, zero))

        def k_body(j, mx):
            slot = slot_of(n_q + j)
            wait(kvbuf, slot)
            advance(j, n_kv, n_q, issue_k, issue_v)
            g, i = j // NI, lax.rem(j, NI)
            new = []
            for b in range(2):
                q8 = q_scr[b, g].astype(jnp.bfloat16)
                sel = zero
                if compute:
                    for h in range(HG):
                        res = lax.dot_general(q8, kvbuf[slot, b, h], NT, preferred_element_type=jnp.float32)
                        sel = res if h == 0 else jnp.where(row == h, res, sel)
                sel = sel * scale
                s_scr[b, j] = sel
                m = jnp.where(i == 0, sel, jnp.maximum(mx[b], sel))
                m_scr[b, g] = m
                new.append(m)
            return tuple(new)
        lax.fori_loop(0, n_kv, k_body, (zero, zero))

        for b in range(2):
            for g in range(G):
                m_scr[b, g] = jnp.broadcast_to(jnp.max(m_scr[b, g], axis=1, keepdims=True), (HG, T))

        def v_body(j, carry):
            slot = slot_of(n_q + n_kv + j)
            wait(kvbuf, slot)
            advance(j, n_kv, n_q + n_kv, issue_v, issue_wo)
            g, i = j // NI, lax.rem(j, NI)
            new = []
            for b in range(2):
                l, acc = carry[b]
                p = jnp.exp(s_scr[b, j] - m_scr[b, g])
                p8 = p.astype(jnp.bfloat16)
                sel = zero
                if compute:
                    for h in range(HG):
                        res = jnp.dot(p8, kvbuf[slot, b, h], preferred_element_type=jnp.float32)
                        sel = res if h == 0 else jnp.where(row == h, res, sel)
                l = jnp.where(i == 0, p, l + p)
                acc = jnp.where(i == 0, sel, acc + sel)

                @pl.when(i == NI - 1)
                def _():
                    o_scr[b, g] = acc / jnp.sum(l, axis=1, keepdims=True)
                new.append((l, acc))
            return tuple(new)
        lax.fori_loop(0, n_kv, v_body, ((zero, zero), (zero, zero)))

        row_d = lax.broadcasted_iota(jnp.int32, (HG, D), 0)

        def o_body(j, acc):
            slot = slot_of(n_q + 2 * n_kv + j)
            wait(wobuf, slot)
            advance(j, n_o, n_q + 2 * n_kv, issue_wo, None)
            g = j // (HG // 2)
            new = []
            for b in range(2):
                a = acc[b]
                o8 = o_scr[b, g].astype(jnp.bfloat16)
                if compute:
                    for hh in range(2):
                        h = lax.rem(j, HG // 2) * 2 + hh
                        res = jnp.dot(o8, wobuf[slot, b, pl.ds(hh * T, T)], preferred_element_type=jnp.float32)
                        a = a + jnp.where(row_d == h, res, 0.0)
                new.append(a)
            return tuple(new)
        zd = jnp.zeros((HG, D), jnp.float32)
        acc = lax.fori_loop(0, n_o, o_body, (zd, zd))
        for b in range(2):
            out_ref[:, b * D:(b + 1) * D] = jnp.sum(acc[b], axis=0, keepdims=True).astype(out_ref.dtype)

    def fn(A_x, A_k_cache, A_v_cache, A_wq, A_wo, B_x, B_k_cache, B_v_cache, B_wq, B_wo):
        _, H, S, Dh = A_k_cache.shape
        D = A_x.shape[-1]
        kv = lambda a: a.reshape(H, S, Dh)
        G = H // HG
        out = pl.pallas_call(
            kernel,
            in_specs=[pl.BlockSpec(memory_space=pl.ANY)] * 10,
            out_specs=pl.BlockSpec(memory_space=pltpu.VMEM),
            out_shape=jax.ShapeDtypeStruct((1, 2 * D), jnp.bfloat16),
            scratch_shapes=[
                pltpu.VMEM((nslot, 2, HG, T, T), jnp.bfloat16),
                pltpu.VMEM((nslot, 2, T, HG * T), jnp.bfloat16),
                pltpu.VMEM((nslot, 2, 2 * T, D), jnp.bfloat16),
                pltpu.VMEM((2, 1, D), jnp.bfloat16),
                pltpu.VMEM((2, G, HG, T), jnp.float32),
                pltpu.VMEM((2, G * (S // T), HG, T), jnp.float32),
                pltpu.VMEM((2, G, HG, T), jnp.float32),
                pltpu.VMEM((2, G, HG, T), jnp.float32),
                pltpu.SemaphoreType.DMA((nslot, 2)),
                pltpu.SemaphoreType.DMA((2,)),
            ],
            compiler_params=pltpu.CompilerParams(vmem_limit_bytes=64 * 2**20, disable_bounds_checks=True),
        )(A_x.reshape(1, D), kv(A_k_cache), kv(A_v_cache), A_wq, A_wo,
          B_x.reshape(1, D), kv(B_k_cache), kv(B_v_cache), B_wq, B_wo)
        return out.reshape(1, 1, 2 * D)
    return fn


_impl = make(rows=64)


@jax.jit
def pallas_concat_heads__mha_block_cached__gqa_block_cached__decode_kernel(
    A_x, A_k_cache, A_v_cache, A_wq, A_wo, B_x, B_k_cache, B_v_cache, B_wq, B_wo,
):
    return _impl(A_x, A_k_cache, A_v_cache, A_wq, A_wo, B_x, B_k_cache, B_v_cache, B_wq, B_wo)
```

```python
import functools

import jax
import jax.numpy as jnp
from jax import lax
import jax.experimental.pallas as pl
import jax.experimental.pallas.tpu as pltpu

T = 128
HG = 8
G = 4
D = 512
NR = 8
NW = 4
LAG = 26
DEPTH = 3
NSLOT = 4
LAST = 2

F32, BF16 = jnp.float32, jnp.bfloat16


def _ds(start, size, multiple):
    return pl.ds(start if isinstance(start, int) else pl.multiple_of(start, multiple), size)


def _wait(buf, sem):
    pltpu.make_async_copy(buf, buf, sem).wait()


def _stream(ax, ak, av, awq, awo, bx, bk, bv, bwq, bwo, out_copy,
            kv_buf, wq_buf, wo_buf, x_buf, x_scr, q_scr, s_scr, m_scr, l_scr, o_scr, y_scr, col_scr, out_buf,
            sem, last_sem, x_sem):
    ni = ak.shape[2] // T
    nb = 2 * NW + 2 * ni

    def wq_piece(w, slot, j, p, main):
        r, half, u = p % NR, p // NR % 2, p // (2 * NR)
        cols = pl.ds(half * 2048, 1792) if main else pl.ds(half * 2048 + 1792, 256)
        return w.at[r, _ds(j * 16 + u * 8, 8, 8), cols], wq_buf.at[j, r, pl.ds(u * 8, 8), cols]

    def kv_piece(cache, slot, j, p, main):
        g, half, quad = p // 4, p // 2 % 2, p % 2
        heads = pl.ds(4 * quad, 3) if main else pl.ds(4 * quad + 3, 1)
        return cache.at[g, heads, _ds(j * T + half * 64, 64, 64)], kv_buf.at[slot, g, heads, pl.ds(half * 64, 64)]

    def wo_piece(w, slot, j, p, main):
        r, c = p % NR, p // NR
        lo, n = (c * 32, 24) if main else (c * 32 + 24, 8)
        return w.at[r, _ds(j * T + lo, n, 8)], wo_buf.at[j, r, pl.ds(lo, n)]

    phases = []
    for b, (wq, k, v, wo) in enumerate(((awq, ak, av, awo), (bwq, bk, bv, bwo))):
        phases += [(wq_piece, wq, b * nb, NW, 32), (kv_piece, k, b * nb + NW, ni, 16),
                   (kv_piece, v, b * nb + NW + ni, ni, 16), (wo_piece, wo, b * nb + NW + 2 * ni, NW, 32)]

    def start(phase, j, p, main):
        piece, array, first, _, _ = phase
        slot = (first + j) & (NSLOT - 1)
        is_last = isinstance(j, int) and first + j == 2 * nb - 1
        pltpu.make_async_copy(*piece(array, slot, j, p, main),
                              last_sem.at[p // LAST] if is_last else sem.at[slot]).start(priority=int(main))

    def start_sliver_from_end(phase, back):
        start(phase, *divmod(phase[3] * phase[4] - back, phase[4]), False)

    def start_step(k, j):
        per = phases[k][4]
        for p in range(per):
            start(phases[k], j, p, True)
            if not isinstance(j, int) or j * per + p >= LAG:
                start(phases[k], j + (p - LAG) // per, (p - LAG) % per, False)
            elif k > 0:
                start_sliver_from_end(phases[k - 1], LAG - j * per - p)

    def start_copies(t):
        for k, (_, _, first, steps, per) in enumerate(phases):
            lo = pl.cdiv(LAG, per)
            hi = steps - (k == len(phases) - 1)
            for j in [*range(lo), *range(hi, steps)]:
                if first + j > 0:
                    pl.when(t == first + j)(functools.partial(start_step, k, j))
            pl.when(jnp.logical_and(t >= first + lo, t < first + hi))(functools.partial(start_step, k, t - first))

        @pl.when(t == 2 * nb)
        def _():
            for back in range(LAG, 0, -1):
                start_sliver_from_end(phases[-1], back)

    def own_rows(results):
        row = lax.broadcasted_iota(jnp.int32, (HG, T), 0)
        out = results[0]
        for h in range(1, HG):
            out = jnp.where(row == h, results[h], out)
        return out

    def q_step(b, j, slot):
        @pl.when(j == 0)
        def _():
            _wait(x_buf.at[b], x_sem.at[b])
            x = jnp.broadcast_to(x_buf[b].astype(F32), (HG, D))
            for s in range(NW):
                x_scr[s] = jnp.concatenate([x[:, 64 * r + 16 * s:64 * r + 16 * s + 16] for r in range(NR)], axis=1)
            q_scr[...] = jnp.zeros(q_scr.shape, F32)
            m_scr[...] = jnp.full(m_scr.shape, -jnp.inf, F32)
            l_scr[...] = jnp.zeros(l_scr.shape, F32)
            o_scr[...] = jnp.zeros(o_scr.shape, F32)
            y_scr[...] = jnp.zeros(y_scr.shape, F32)

        _wait(wq_buf.at[j], sem.at[slot])
        x = x_scr[j].astype(BF16)
        for g in range(G):
            w = wq_buf[j, :, :, g * HG * T:(g + 1) * HG * T].reshape(T, HG * T)
            q = jnp.dot(x, w, preferred_element_type=F32)
            q_scr[g] += own_rows([q[:, h * T:(h + 1) * T] for h in range(HG)])

    def k_step(j, slot):
        _wait(kv_buf.at[slot], sem.at[slot])
        for g in range(G):
            q = q_scr[g].astype(BF16)
            s = own_rows([lax.dot_general(q, kv_buf[slot, g, h], (((1,), (1,)), ((), ())),
                                          preferred_element_type=F32) for h in range(HG)]) * T ** -0.5
            s_scr[j, g] = s
            m_scr[g] = jnp.maximum(m_scr[g], s)

        @pl.when(j == ni - 1)
        def _():
            for g in range(G):
                m_scr[g] = jnp.broadcast_to(jnp.max(m_scr[g], axis=1, keepdims=True), (HG, T))

    def v_step(j, slot):
        _wait(kv_buf.at[slot], sem.at[slot])
        for g in range(G):
            p = jnp.exp(s_scr[j, g] - m_scr[g])
            l_scr[g] += p
            p = p.astype(BF16)
            o_scr[g] += own_rows([jnp.dot(p, kv_buf[slot, g, h], preferred_element_type=F32) for h in range(HG)])

        @pl.when(j == ni - 1)
        def _():
            for g in range(G):
                o_scr[g] = o_scr[g] / jnp.sum(l_scr[g], axis=1, keepdims=True)

    def o_step(j, slot):
        _wait(wo_buf.at[j], sem.at[slot])
        row = lax.broadcasted_iota(jnp.int32, (HG, D), 0)
        y = y_scr[...]
        for r in range(NR):
            part = jnp.dot(o_scr[r // 2].astype(BF16), wo_buf[j, r], preferred_element_type=F32)
            y += jnp.where(row == r % 2 * NW + j, part, 0.0)
        y_scr[...] = y

        @pl.when(j < 2)
        def _():
            for e in range(NR // 2):
                o = o_scr[2 * j + e // 2, pl.ds(e % 2 * NW + NW - 1, 1), :].astype(BF16).astype(F32)
                col_scr[NR // 2 * j + e] = jnp.broadcast_to(o, (T, T)).T

        @pl.when(j == NW - 1)
        def _():
            out_buf[:, :D] = jnp.sum(y, axis=0, keepdims=True).astype(BF16)

    def body(ahead, carry):
        start_copies(ahead)

        @pl.when(ahead >= DEPTH)
        def _():
            t = ahead - DEPTH
            b = (t >= nb).astype(jnp.int32)
            u = t - b * nb
            slot = t & (NSLOT - 1)
            pl.when(u < NW)(lambda: q_step(b, u, slot))
            pl.when(jnp.logical_and(u >= NW, u < NW + ni))(lambda: k_step(u - NW, slot))
            pl.when(jnp.logical_and(u >= NW + ni, u < NW + 2 * ni))(lambda: v_step(u - (NW + ni), slot))
            pl.when(u >= NW + 2 * ni)(lambda: o_step(u - (NW + 2 * ni), slot))
        return carry

    start_step(0, 0)
    for b, x in enumerate((ax, bx)):
        pltpu.make_async_copy(x, x_buf.at[b], x_sem.at[b]).start()
    lax.fori_loop(1, 2 * nb - 1 + DEPTH, body, None)

    y = y_scr[...]
    for p in range(32):
        r, rows = p % NR, pl.ds(p // NR * 32, 32)
        if p % LAST == 0:
            _wait(wo_buf.at[NW - 1, pl.ds(r, LAST), rows], last_sem.at[p // LAST])
        part = wo_buf[NW - 1, r, rows].astype(F32) * jnp.concatenate([col_scr[r, rows]] * (D // T), axis=1)
        y += (part[0:8] + part[8:16]) + (part[16:24] + part[24:32])
    out_buf[:, D:] = jnp.sum(y, axis=0, keepdims=True).astype(BF16)
    out_copy.start()


def _kernel(*refs):
    inputs, out, scratch, out_sem = refs[:10], refs[10], refs[11:-1], refs[-1]
    out_copy = pltpu.make_async_copy(scratch[-1], out, out_sem)
    pl.run_scoped(functools.partial(_stream, *inputs, out_copy, *scratch),
                  pltpu.SemaphoreType.DMA((NSLOT,)),
                  pltpu.SemaphoreType.DMA((32 // LAST,)),
                  pltpu.SemaphoreType.DMA((2,)))
    out_copy.wait()


@jax.jit
def pallas_concat_heads__mha_block_cached__gqa_block_cached__decode_kernel(
    A_x: jax.Array,
    A_k_cache: jax.Array,
    A_v_cache: jax.Array,
    A_wq: jax.Array,
    A_wo: jax.Array,
    B_x: jax.Array,
    B_k_cache: jax.Array,
    B_v_cache: jax.Array,
    B_wq: jax.Array,
    B_wo: jax.Array,
):
    keys = A_k_cache.shape[2]
    assert keys % T == 0 and keys >= 2 * T

    def block(x, k, v, wq, wo):
        assert x.shape == (1, 1, D) and k.shape == v.shape == (1, G * HG, keys, T)
        assert wq.shape == (D, G * HG * T) and wo.shape == (G * HG * T, D)
        return (x.reshape(1, D), k.reshape(G, HG, keys, T), v.reshape(G, HG, keys, T),
                wq.reshape(NR, D // NR, G * HG * T), wo.reshape(NR, NW * T, D))

    out = pl.pallas_call(
        _kernel,
        in_specs=[pl.BlockSpec(memory_space=pl.ANY)] * 10,
        out_specs=pl.BlockSpec(memory_space=pl.ANY),
        out_shape=jax.ShapeDtypeStruct((1, 2 * D), BF16),
        scratch_shapes=[
            pltpu.VMEM((NSLOT, G, HG, T, T), BF16),
            pltpu.VMEM((NW, NR, T // NR, G * HG * T), BF16),
            pltpu.VMEM((NW, NR, T, D), BF16),
            pltpu.VMEM((2, 1, D), BF16),
            pltpu.VMEM((NW, HG, T), F32),
            pltpu.VMEM((G, HG, T), F32),
            pltpu.VMEM((keys // T, G, HG, T), F32),
            pltpu.VMEM((G, HG, T), F32),
            pltpu.VMEM((G, HG, T), F32),
            pltpu.VMEM((G, HG, T), F32),
            pltpu.VMEM((HG, D), F32),
            pltpu.VMEM((NR, T, T), F32),
            pltpu.VMEM((1, 2 * D), BF16),
            pltpu.SemaphoreType.DMA(()),
        ],
        compiler_params=pltpu.CompilerParams(vmem_limit_bytes=32 * 2**20),
    )(*block(A_x, A_k_cache, A_v_cache, A_wq, A_wo), *block(B_x, B_k_cache, B_v_cache, B_wq, B_wo))
    return out.reshape(1, 1, 2 * D)
```
